```python
import os as _os
_os.environ.setdefault("JAX_PLATFORMS", "cpu")
import jax
import jax.numpy as jnp

def _softmax(x, axis=-1):
    return jax.nn.softmax(x, axis=axis)
def _gelu(x):
    return jax.nn.gelu(x, approximate=True)
def _silu(x):
    return jax.nn.silu(x)
def _sigmoid(x):
    return jax.nn.sigmoid(x)
def _layernorm(x, axis=-1, eps=1e-5):
    m = jnp.mean(x, axis=axis, keepdims=True)
    v = jnp.var(x, axis=axis, keepdims=True)
    return (x - m) / jnp.sqrt(v + eps)
def _scatter_add(tgt, idx, src, axis=0):
    return tgt.at[idx].add(src)
def _segment_sum(src, seg, n):
    return jax.ops.segment_sum(src, seg, n)
class _Rng:
    def __init__(self, key):
        self._k = key
    def _next(self):
        self._k, sub = jax.random.split(self._k)
        return sub
    def normal(self, shape):
        return jax.random.normal(self._next(), shape, dtype=jnp.bfloat16)
    def randint(self, lo, hi, shape):
        return jax.random.randint(self._next(), shape, lo, hi, dtype=jnp.int32)
    def uniform(self, shape, lo=0.0, hi=1.0):
        return jax.random.uniform(self._next(), shape, jnp.bfloat16, lo, hi)
    def permutation(self, n):
        return jax.random.permutation(self._next(), n)


kernel_name = 'parallel_sum__ssm_conv_s5__glu_gated_swiglu__prompt'

def setup_inputs():
    _rng = _Rng(jax.random.key(int.from_bytes(__import__("os").urandom(4), "little")))
    _w = (lambda a: (lambda t: t.astype(jnp.bfloat16) if jnp.issubdtype(t.dtype, jnp.floating) else t)(jnp.asarray(a)))
    def _A_setup():
        B, S, D = 1, 2048, 640
        P = D
        Lambda_re = -0.5 * jnp.exp((lambda *s: _rng.normal(s) * 0.4)(P))
        Lambda_im = (lambda *s: _rng.normal(s) * 0.4)(P) * 1.0
        B_re = (lambda *s: _rng.normal(s) * 0.4)(P, D) * (D ** -0.5)
        B_im = (lambda *s: _rng.normal(s) * 0.4)(P, D) * (D ** -0.5)
        C_re = (lambda *s: _rng.normal(s) * 0.4)(D, P) * (P ** -0.5)
        C_im = (lambda *s: _rng.normal(s) * 0.4)(D, P) * (P ** -0.5)
        log_dt = (lambda *s: _rng.normal(s) * 0.4)(P) * 0.3 - 2.0
        Dskip = (lambda *s: _rng.normal(s) * 0.4)(D)
        return {
            "x": _w((lambda *s: _rng.normal(s) * 0.05)(B, S, D)),
            "Lambda_re": _w(Lambda_re),
            "Lambda_im": _w(Lambda_im),
            "B_re": _w(B_re),
            "B_im": _w(B_im),
            "C_re": _w(C_re),
            "C_im": _w(C_im),
            "log_dt": _w(log_dt),
            "Dskip": _w(Dskip),
        }
    _A_in = _A_setup()

    def _B_setup():
        B, S, D, F = 1, 2048, 640, 1728
        return {
            "x": _w((lambda *s: _rng.normal(s) * 0.05)(B, S, D)),
            "w1": _w((lambda *s: _rng.normal(s) * 0.1)(D, F) * (2.0 / D) ** 0.5),
            "w3": _w((lambda *s: _rng.normal(s) * 0.1)(D, F) * (2.0 / D) ** 0.5),
            "w2": _w((lambda *s: _rng.normal(s) * 0.1)(F, D) * (2.0 / F) ** 0.5),
        }
    _B_in = _B_setup()

    return {
        "A_x": _A_in["x"],
        "A_Lambda_re": _A_in["Lambda_re"],
        "A_Lambda_im": _A_in["Lambda_im"],
        "A_B_re": _A_in["B_re"],
        "A_B_im": _A_in["B_im"],
        "A_C_re": _A_in["C_re"],
        "A_C_im": _A_in["C_im"],
        "A_log_dt": _A_in["log_dt"],
        "A_Dskip": _A_in["Dskip"],
        "B_x": _B_in["x"],
        "B_w1": _B_in["w1"],
        "B_w3": _B_in["w3"],
        "B_w2": _B_in["w2"],
    }

def reference(A_x, A_Lambda_re, A_Lambda_im, A_B_re, A_B_im, A_C_re, A_C_im, A_log_dt, A_Dskip, B_x, B_w1, B_w3, B_w2):
    def _A_ref(x, Lambda_re, Lambda_im, B_re, B_im, C_re, C_im, log_dt, Dskip):
        Bsz, L, H = x.shape
        Lam = Lambda_re + 1j * Lambda_im
        Bmat = B_re + 1j * B_im
        Cmat = C_re + 1j * C_im
        dt = jnp.exp(log_dt)
        Lam_bar = jnp.exp(dt * Lam)
        B_bar = ((Lam_bar - 1.0) / Lam)[:, None] * Bmat
        Bu = jnp.einsum("bld,pd->blp", x + 0j, B_bar)
        h = jnp.zeros_like(Bu[:, 0, :])
        hs = []
        for t in range(L):
            h = Lam_bar[None, :] * h + Bu[:, t, :]
            hs.append(h)
        hseq = jnp.stack(hs, 1)
        y = 2.0 * jnp.einsum("blp,dp->bld", hseq, Cmat).real + x * Dskip[None, None, :]
        return y

    def _B_ref(x, w1, w3, w2):
        gate = jnp.einsum("bsd,df->bsf", x, w1)
        up = jnp.einsum("bsd,df->bsf", x, w3)
        h = _silu(gate) * up
        out = jnp.einsum("bsf,fd->bsd", h, w2)
        return out

    x = A_x
    xn = _layernorm(x, axis=-1)
    return x + _A_ref(xn, A_Lambda_re, A_Lambda_im, A_B_re, A_B_im, A_C_re, A_C_im, A_log_dt, A_Dskip) + _B_ref(xn, B_w1, B_w3, B_w2)
```

```python
import jax
import jax.numpy as jnp
import jax.experimental.pallas as pl
import jax.experimental.pallas.tpu as pltpu

F32 = jnp.float32
BF16 = jnp.bfloat16
TM = 256
UNROLL = False
PAD = 4
PIPE = True


def _cmul(ar, ai, br, bi):
    return ar * br - ai * bi, ar * bi + ai * br


def _nt(a, b):
    return jax.lax.dot_general(a, b, (((1,), (1,)), ((), ())), preferred_element_type=F32)


def _nn(a, b):
    return jnp.dot(a, b, preferred_element_type=F32)


def kern(x_hbm, lr_ref, li_ref, bre_hbm, bim_hbm, cre_hbm, cim_hbm, ldt_ref, dsk_ref,
         w1_hbm, w3_hbm, w2_hbm, o_hbm,
         x_v, wa_v, w2_v, xp_v, c2_v, o_v, co_ref, carry_ref, h_ref, hh_ref, xn_v, base_v, sem, osem):
    S, D = x_hbm.shape
    F = w1_hbm.shape[0]
    NB = S // TM
    NT = F // 128
    R = F - NT * 128
    cp = []

    def add(src, dst):
        cp.append(pltpu.make_async_copy(src, dst, sem.at[len(cp)]))
        return cp[-1]

    d_x0 = add(x_hbm.at[0:TM], x_v.at[0:TM])
    g0 = 2 * D
    d_gu = []
    d_b = None
    for t in range(0, NT, 2):
        n = min(2, NT - t) * 128
        a = add(w1_hbm.at[t * 128:t * 128 + n], wa_v.at[g0 + 2 * t * 128:g0 + 2 * t * 128 + n])
        b = add(w3_hbm.at[t * 128:t * 128 + n], wa_v.at[g0 + 2 * t * 128 + n:g0 + 2 * t * 128 + 2 * n])
        d_gu.append((t, n, a, b))
        if t == 0:
            d_b = (add(bre_hbm, wa_v.at[0:D]), add(bim_hbm, wa_v.at[D:2 * D]))
    r0 = g0 + 2 * NT * 128
    d_r = (add(w1_hbm.at[NT * 128:F], wa_v.at[r0:r0 + R]), add(w3_hbm.at[NT * 128:F], wa_v.at[r0 + R:r0 + 2 * R]))
    d_c = (add(cre_hbm, c2_v.at[:, 0:D]), add(cim_hbm, c2_v.at[:, D:2 * D]))
    d_w2 = add(w2_hbm, w2_v)
    d_x1 = add(x_hbm.at[TM:2 * TM], x_v.at[TM:2 * TM])
    d_x2 = add(x_hbm.at[2 * TM:S], x_v.at[2 * TM:S])
    for c in cp:
        c.start()

    def vec(ref):
        return jnp.broadcast_to(ref[...].astype(F32).reshape(1, D), (8, D))

    lr = vec(lr_ref)
    li = vec(li_ref)
    dt = jnp.exp(vec(ldt_ref)).astype(BF16).astype(F32)
    mag = jnp.exp(dt * lr)
    ar = mag * jnp.cos(dt * li)
    ai = mag * jnp.sin(dt * li)
    den = lr * lr + li * li
    cr = ((ar - 1.0) * lr + ai * li) / den
    ci = (ai * lr - (ar - 1.0) * li) / den
    row = jax.lax.broadcasted_iota(jnp.int32, (8, D), 0)
    ai = -ai
    co_ref[0] = ar
    co_ref[1] = ai
    qr, qi = ar, ai
    for _ in range(5):
        qr, qi = _cmul(qr, qi, qr, qi)
    for n in range(3):
        co_ref[2 + 2 * n] = qr
        co_ref[3 + 2 * n] = qi
        qr, qi = _cmul(qr, qi, qr, qi)
    co_ref[9] = 2.0 * cr
    co_ref[10] = 2.0 * ci
    co_ref[8] = vec(dsk_ref)
    carry_ref[...] = jnp.zeros_like(carry_ref)

    def ocopy(b):
        return pltpu.make_async_copy(o_v.at[b % 2], o_hbm.at[pl.ds(pl.multiple_of(b * TM, TM), TM)], osem.at[b % 2])

    def ln(b):
        T = TM // 8
        Q = T + PAD
        x0 = x_v[pl.ds(pl.multiple_of(b * TM, TM), TM), :].astype(F32)
        for c in range(5):
            for g in range(8):
                xp_v[c, g * Q:g * Q + T, :] = x0[g * T:(g + 1) * T, c * 128:(c + 1) * 128]
        x = jnp.concatenate([jnp.concatenate([xp_v[c, pl.ds(i, 8, stride=Q), :] for i in range(T)], 0)
                             for c in range(5)], 1)
        m = jnp.mean(x, axis=-1, keepdims=True)
        xc = x - m
        v = jnp.mean(xc * xc, axis=-1, keepdims=True)
        xn32 = xc * jax.lax.rsqrt(v + 1e-5)
        xn = xn32.astype(BF16)
        xn_v[...] = xn
        base_v[...] = x + xn32 * co_ref[8, 0:1, :]

    def block(b, first):
        def w(*ds):
            if first:
                for d in ds:
                    d.wait()
        w(d_x0)
        T = TM // 8
        Q = T + PAD
        if first or not PIPE:
            ln(b)
        xn = xn_v[...]
        base = base_v[...]

        def glu(t, n, a, b_):
            o = g0 + 2 * t * 128
            g = _nt(xn, wa_v[o:o + n])
            u = _nt(xn, wa_v[o + n:o + 2 * n])
            hh_ref[:, t * 128:t * 128 + n] = (g * jax.nn.sigmoid(g) * u).astype(BF16)

        w(*d_gu[0][2:])
        if first:
            for c in ():
                c.start()
        glu(*d_gu[0])
        w(*d_b, *d_gu[1][2:], *d_gu[2][2:])
        if first:
            for c in ():
                c.start()
        bur = _nt(xn, wa_v[0:D])
        bui = _nt(xn, wa_v[D:2 * D])

        def scan(c):
            ls = slice(c * 128, (c + 1) * 128)
            co = [co_ref[k, :, ls] for k in range(11)]
            us = []
            for j in range(T):
                p, q = bur[j * 8:(j + 1) * 8, ls], bui[j * 8:(j + 1) * 8, ls]
                us.append((co[9] * p - co[10] * q, -(co[9] * q) - co[10] * p))
            r, i = us[0]
            for j in range(1, T):
                tr, ti = _cmul(co[0], co[1], r, i)
                r, i = tr + us[j][0], ti + us[j][1]
            sub = jax.lax.broadcasted_iota(jnp.int32, (8, 128), 0)
            r = jnp.where(sub == 0, carry_ref[0, :, ls], pltpu.roll(r, 1, 0))
            i = jnp.where(sub == 0, carry_ref[1, :, ls], pltpu.roll(i, 1, 0))
            for n in range(3):
                tr, ti = _cmul(co[2 + 2 * n], co[3 + 2 * n], pltpu.roll(r, 1 << n, 0), pltpu.roll(i, 1 << n, 0))
                r = jnp.where(sub >= (1 << n), r + tr, r)
                i = jnp.where(sub >= (1 << n), i + ti, i)
            hr, hi = [], []
            for j in range(T):
                tr, ti = _cmul(co[0], co[1], r, i)
                r, i = tr + us[j][0], ti + us[j][1]
                hr.append(r)
                hi.append(i)
            h_ref[:, ls] = jnp.concatenate(hr, 0).astype(BF16)
            h_ref[:, D + c * 128:D + (c + 1) * 128] = jnp.concatenate(hi, 0).astype(BF16)
            carry_ref[0, :, ls] = pltpu.roll(r, 1, 0)
            carry_ref[1, :, ls] = pltpu.roll(i, 1, 0)

        for k in range(1, len(d_gu)):
            if k == 3:
                w(*d_r, *[d for g in d_gu[3:] for d in g[2:]])
            glu(*d_gu[k])
            if k - 1 < D // 128:
                scan(k - 1)
        gu = _nt(xn, wa_v[r0:r0 + 2 * R])
        u = pltpu.roll(gu, R, 1)
        hh_ref[:, NT * 128:F] = (gu * jax.nn.sigmoid(gu) * u)[:, :R].astype(BF16)
        w(*d_c, d_w2, d_x1)
        if PIPE:
            ln(jnp.minimum(b + 1, NB - 1))
        y = base + _nn(hh_ref[...], w2_v[...]) + _nt(h_ref[...], c2_v[...])
        for i in range(T):
            for c in range(5):
                xp_v[5 + c, pl.ds(i, 8, stride=Q), :] = y[8 * i:8 * i + 8, c * 128:(c + 1) * 128]
        for c in range(5):
            for g in range(8):
                o_v[b % 2, g * T:(g + 1) * T, c * 128:(c + 1) * 128] = xp_v[5 + c, g * Q:g * Q + T, :]
        ocopy(b).start()

    block(0, True)
    d_x2.wait()
    if UNROLL:
        for b in range(1, NB):
            if b >= 2:
                ocopy(b - 2).wait()
            block(b, False)
    else:
        def body(b, _):
            @pl.when(b >= 2)
            def _():
                ocopy(b - 2).wait()
            block(b, False)
        jax.lax.fori_loop(1, NB, body, None)
    ocopy(NB - 2).wait()
    ocopy(NB - 1).wait()


@jax.jit
def pallas_parallel_sum__ssm_conv_s5__glu_gated_swiglu__prompt_kernel(A_x, A_Lambda_re, A_Lambda_im, A_B_re, A_B_im, A_C_re, A_C_im, A_log_dt, A_Dskip, B_x, B_w1, B_w3, B_w2):
    B, S, D = A_x.shape
    F = B_w1.shape[1]
    x = A_x.reshape(S, D)
    H = pl.BlockSpec(memory_space=pltpu.HBM)
    V = pl.BlockSpec(memory_space=pltpu.VMEM)
    args = (x, A_Lambda_re, A_Lambda_im, A_B_re, A_B_im, A_C_re, A_C_im, A_log_dt, A_Dskip, B_w1.T, B_w3.T, B_w2)
    out = pl.pallas_call(
        kern,
        in_specs=[H, V, V, H, H, H, H, V, V, H, H, H],
        out_specs=H,
        out_shape=jax.ShapeDtypeStruct((S, D), F32),
        scratch_shapes=[pltpu.VMEM((S, D), BF16), pltpu.VMEM((2 * D + 2 * F, D), BF16), pltpu.VMEM((F, D), BF16),
                        pltpu.VMEM((10, TM + 9 * PAD + TM // 8, 128), F32), pltpu.VMEM((D, 2 * D), BF16), pltpu.VMEM((2, TM, D), F32),
                        pltpu.VMEM((11, 8, D), F32), pltpu.VMEM((2, 8, D), F32),
                        pltpu.VMEM((TM, 2 * D), BF16), pltpu.VMEM((TM, F), BF16), pltpu.VMEM((TM, D), BF16), pltpu.VMEM((TM, D), F32),
                        pltpu.SemaphoreType.DMA((32,)), pltpu.SemaphoreType.DMA((2,))],
        compiler_params=pltpu.CompilerParams(vmem_limit_bytes=100 * 1024 * 1024),
    )(*args)
    return out.reshape(B, S, D)
```
